```python
import os as _os
_os.environ.setdefault("JAX_PLATFORMS", "cpu")
import jax
import jax.numpy as jnp

def _softmax(x, axis=-1):
    return jax.nn.softmax(x, axis=axis)
def _gelu(x):
    return jax.nn.gelu(x, approximate=True)
def _silu(x):
    return jax.nn.silu(x)
def _sigmoid(x):
    return jax.nn.sigmoid(x)
def _layernorm(x, axis=-1, eps=1e-5):
    m = jnp.mean(x, axis=axis, keepdims=True)
    v = jnp.var(x, axis=axis, keepdims=True)
    return (x - m) / jnp.sqrt(v + eps)
def _scatter_add(tgt, idx, src, axis=0):
    return tgt.at[idx].add(src)
def _segment_sum(src, seg, n):
    return jax.ops.segment_sum(src, seg, n)
class _Rng:
    def __init__(self, key):
        self._k = key
    def _next(self):
        self._k, sub = jax.random.split(self._k)
        return sub
    def normal(self, shape):
        return jax.random.normal(self._next(), shape, dtype=jnp.bfloat16)
    def randint(self, lo, hi, shape):
        return jax.random.randint(self._next(), shape, lo, hi, dtype=jnp.int32)
    def uniform(self, shape, lo=0.0, hi=1.0):
        return jax.random.uniform(self._next(), shape, jnp.bfloat16, lo, hi)
    def permutation(self, n):
        return jax.random.permutation(self._next(), n)


kernel_name = 'concat_heads__gqa_block_cached__gqa_block_cached__near_ridge'

def setup_inputs():
    _rng = _Rng(jax.random.key(int.from_bytes(__import__("os").urandom(4), "little")))
    _w = (lambda a: (lambda t: t.astype(jnp.bfloat16) if jnp.issubdtype(t.dtype, jnp.floating) else t)(jnp.asarray(a)))
    def _A_setup():
        B, Sq, D = 8, 240, 640
        Hq, Hkv, Sk, Dh = 32, 32, 1024, 192
        assert Hq % Hkv == 0, (Hq, Hkv)
        return {
            "x": _w((lambda *s: _rng.normal(s) * 0.8)(B, Sq, D)),
            "k_cache": _w((lambda *s: _rng.normal(s) * 0.8)(B, Hkv, Sk, Dh)),
            "v_cache": _w((lambda *s: _rng.normal(s) * 0.05)(B, Hkv, Sk, Dh)),
            "wq": _w((lambda *s: _rng.normal(s) * 0.8)(D, Hq * Dh) * (D ** -0.5)),
            "wo": _w((lambda *s: _rng.normal(s) * 0.05)(Hq * Dh, D) * ((Hq * Dh) ** -0.5)),
        }
    _A_in = _A_setup()

    def _B_setup():
        B, Sq, D = 8, 240, 640
        Hq, Hkv, Sk, Dh = 32, 32, 1024, 192
        assert Hq % Hkv == 0, (Hq, Hkv)
        return {
            "x": _w((lambda *s: _rng.normal(s) * 0.8)(B, Sq, D)),
            "k_cache": _w((lambda *s: _rng.normal(s) * 0.8)(B, Hkv, Sk, Dh)),
            "v_cache": _w((lambda *s: _rng.normal(s) * 0.05)(B, Hkv, Sk, Dh)),
            "wq": _w((lambda *s: _rng.normal(s) * 0.8)(D, Hq * Dh) * (D ** -0.5)),
            "wo": _w((lambda *s: _rng.normal(s) * 0.05)(Hq * Dh, D) * ((Hq * Dh) ** -0.5)),
        }
    _B_in = _B_setup()

    return {
        "A_x": _A_in["x"],
        "A_k_cache": _A_in["k_cache"],
        "A_v_cache": _A_in["v_cache"],
        "A_wq": _A_in["wq"],
        "A_wo": _A_in["wo"],
        "B_x": _B_in["x"],
        "B_k_cache": _B_in["k_cache"],
        "B_v_cache": _B_in["v_cache"],
        "B_wq": _B_in["wq"],
        "B_wo": _B_in["wo"],
    }

def reference(A_x, A_k_cache, A_v_cache, A_wq, A_wo, B_x, B_k_cache, B_v_cache, B_wq, B_wo):
    def _A_ref(x, k_cache, v_cache, wq, wo):
        B, Sq, D = x.shape
        Hq, Dh = 32, 192
        Hkv = k_cache.shape[1]
        rep = Hq // Hkv
        q = (lambda x, *d: x.transpose(*d))((x @ wq).reshape(B, Sq, Hq, Dh), 0, 2, 1, 3)
        k = jnp.repeat(k_cache, rep, axis=1)
        v = jnp.repeat(v_cache, rep, axis=1)
        scores = jnp.einsum("bhqd,bhkd->bhqk", q, k) * (Dh ** -0.5)
        p = _softmax(scores, axis=-1)
        o = jnp.einsum("bhqk,bhkd->bhqd", p, v)
        return (lambda x, *d: x.transpose(*d))(o, 0, 2, 1, 3).reshape(B, Sq, Hq * Dh) @ wo

    def _B_ref(x, k_cache, v_cache, wq, wo):
        B, Sq, D = x.shape
        Hq, Dh = 32, 192
        Hkv = k_cache.shape[1]
        rep = Hq // Hkv
        q = (lambda x, *d: x.transpose(*d))((x @ wq).reshape(B, Sq, Hq, Dh), 0, 2, 1, 3)
        k = jnp.repeat(k_cache, rep, axis=1)
        v = jnp.repeat(v_cache, rep, axis=1)
        scores = jnp.einsum("bhqd,bhkd->bhqk", q, k) * (Dh ** -0.5)
        p = _softmax(scores, axis=-1)
        o = jnp.einsum("bhqk,bhkd->bhqd", p, v)
        return (lambda x, *d: x.transpose(*d))(o, 0, 2, 1, 3).reshape(B, Sq, Hq * Dh) @ wo

    a = _A_ref(A_x, A_k_cache, A_v_cache, A_wq, A_wo)
    b = _B_ref(B_x, B_k_cache, B_v_cache, B_wq, B_wo)
    return jnp.concatenate([a, b], axis=-1)
```

```python
import functools
import math

import jax
import jax.numpy as jnp
import jax.experimental.pallas as pl
import jax.experimental.pallas.tpu as pltpu


def _attn_kernel(
    ax_ref, ak_ref, av_ref, awq_ref, awo_ref,
    bx_ref, bk_ref, bv_ref, bwq_ref, bwo_ref,
    out_ref,
    aq_scr, bq_scr, ao_scr, bo_scr,
    *, heads_per_step, dh, d_model, scale,
):
    hs = pl.program_id(1)
    nhs = pl.num_programs(1)

    branches = (
        (ax_ref, ak_ref, av_ref, awq_ref, awo_ref, aq_scr, ao_scr, 0),
        (bx_ref, bk_ref, bv_ref, bwq_ref, bwo_ref, bq_scr, bo_scr, 1),
    )

    @pl.when(hs == 0)
    def _():
        for x_ref, _, _, wq_ref, _, q_scr, _, _ in branches:
            q = jnp.dot(x_ref[0], wq_ref[...], preferred_element_type=jnp.float32)
            q = (q * scale).astype(jnp.bfloat16)
            for h in range(q_scr.shape[0]):
                q_scr[h] = q[:, h * dh:(h + 1) * dh]

    for x_ref, k_ref, v_ref, wq_ref, wo_ref, q_scr, o_scr, bi in branches:
        for j in range(heads_per_step):
            h = hs * heads_per_step + j
            q = q_scr[h]
            k = k_ref[0, j]
            v = v_ref[0, j]
            s = jax.lax.dot_general(q, k, (((1,), (1,)), ((), ())),
                                    preferred_element_type=jnp.float32)
            m = jnp.max(s, axis=-1, keepdims=True)
            p = jnp.exp2(s - m)
            l = jnp.sum(p, axis=-1, keepdims=True)
            o = jnp.dot(p.astype(jnp.bfloat16), v, preferred_element_type=jnp.float32)
            o = o / l
            o_scr[h] = o.astype(jnp.bfloat16)

    @pl.when(hs == nhs - 1)
    def _():
        for x_ref, _, _, _, wo_ref, _, o_scr, bi in branches:
            o_all = jnp.concatenate([o_scr[h] for h in range(o_scr.shape[0])], axis=-1)
            y = jnp.dot(o_all, wo_ref[...], preferred_element_type=jnp.float32)
            out_ref[0, :, bi * d_model:(bi + 1) * d_model] = y.astype(out_ref.dtype)


@jax.jit
def pallas_concat_heads__gqa_block_cached__gqa_block_cached__near_ridge_kernel(
    A_x: jax.Array,
    A_k_cache: jax.Array,
    A_v_cache: jax.Array,
    A_wq: jax.Array,
    A_wo: jax.Array,
    B_x: jax.Array,
    B_k_cache: jax.Array,
    B_v_cache: jax.Array,
    B_wq: jax.Array,
    B_wo: jax.Array,
):
    B, Sq, D = A_x.shape
    _, Hkv, Sk, Dh = A_k_cache.shape
    Hq = A_wq.shape[1] // Dh
    assert Hq == Hkv == 32 and Dh == 192
    HPS = 2
    scale = (Dh ** -0.5) * math.log2(math.e)

    x_spec = pl.BlockSpec((1, Sq, D), lambda b, h: (b, 0, 0))
    kv_spec = pl.BlockSpec((1, HPS, Sk, Dh), lambda b, h: (b, h, 0, 0))
    wq_spec = pl.BlockSpec((D, Hq * Dh), lambda b, h: (0, 0), pipeline_mode=pl.Buffered(1))
    wo_spec = pl.BlockSpec((Hq * Dh, D), lambda b, h: (0, 0), pipeline_mode=pl.Buffered(1))
    out_spec = pl.BlockSpec((1, Sq, 2 * D), lambda b, h: (b, 0, 0))

    kernel = functools.partial(_attn_kernel, heads_per_step=HPS, dh=Dh, d_model=D, scale=scale)
    return pl.pallas_call(
        kernel,
        grid=(B, Hq // HPS),
        in_specs=[x_spec, kv_spec, kv_spec, wq_spec, wo_spec,
                  x_spec, kv_spec, kv_spec, wq_spec, wo_spec],
        out_specs=out_spec,
        out_shape=jax.ShapeDtypeStruct((B, Sq, 2 * D), jnp.bfloat16),
        scratch_shapes=[
            pltpu.VMEM((Hq, Sq, Dh), jnp.bfloat16),
            pltpu.VMEM((Hq, Sq, Dh), jnp.bfloat16),
            pltpu.VMEM((Hq, Sq, Dh), jnp.bfloat16),
            pltpu.VMEM((Hq, Sq, Dh), jnp.bfloat16),
        ],
        compiler_params=pltpu.CompilerParams(
            dimension_semantics=("arbitrary", "arbitrary"),
            vmem_limit_bytes=100 * 1024 * 1024,
        ),
    )(A_x, A_k_cache, A_v_cache, A_wq, A_wo, B_x, B_k_cache, B_v_cache, B_wq, B_wo)
```

```python
import functools
import math

import jax
import jax.numpy as jnp
import jax.experimental.pallas as pl
import jax.experimental.pallas.tpu as pltpu


def _attn_kernel(
    ax_ref, ak_ref, av_ref, awq_hbm, awo_hbm,
    bx_ref, bk_ref, bv_ref, bwq_hbm, bwo_hbm,
    out_ref,
    aq_scr, bq_scr, ao_scr, bo_scr,
    awq_ref, awo_ref, bwq_ref, bwo_ref, w_sems,
    *, heads_per_step, dh, d_model, scale,
):
    b = pl.program_id(0)
    hs = pl.program_id(1)
    nhs = pl.num_programs(1)
    n_heads = aq_scr.shape[0]

    branches = (
        (ax_ref, ak_ref, av_ref, awq_ref, awo_ref, aq_scr, ao_scr, 0),
        (bx_ref, bk_ref, bv_ref, bwq_ref, bwo_ref, bq_scr, bo_scr, 1),
    )
    w_copies = [
        pltpu.make_async_copy(src, dst, w_sems.at[i])
        for i, (src, dst) in enumerate(
            ((awq_hbm, awq_ref), (bwq_hbm, bwq_ref), (awo_hbm, awo_ref), (bwo_hbm, bwo_ref)))
    ]

    @pl.when(jnp.logical_and(b == 0, hs == 0))
    def _():
        for c in w_copies:
            c.start()

    @pl.when(hs == 0)
    def _():
        for x_ref, _, _, wq_ref, _, q_scr, _, bi in branches:
            @pl.when(b == 0)
            def _():
                w_copies[bi].wait()
            q = jnp.dot(x_ref[0], wq_ref[...], preferred_element_type=jnp.float32)
            q = (q * scale).astype(jnp.bfloat16)
            for h in range(n_heads):
                q_scr[h] = q[:, h * dh:(h + 1) * dh]

    heads = [(kt_ref, vt_ref, q_scr, o_scr, j)
             for _, kt_ref, vt_ref, _, _, q_scr, o_scr, _ in branches
             for j in range(heads_per_step)]

    def qk(i):
        kt_ref, _, q_scr, _, j = heads[i]
        q = q_scr[hs * heads_per_step + j]
        return jnp.dot(q, kt_ref[0, j], preferred_element_type=jnp.float32)

    def softmax_pv(i, s):
        _, vt_ref, _, o_scr, j = heads[i]
        m = jnp.max(s, axis=-1, keepdims=True)
        p = jnp.exp2(s - m)
        l = jnp.sum(p, axis=-1, keepdims=True)
        ot = jax.lax.dot_general(vt_ref[0, j], p.astype(jnp.bfloat16), (((1,), (1,)), ((), ())),
                                 preferred_element_type=jnp.float32)
        o_scr[hs * heads_per_step + j] = (ot.T / l).astype(jnp.bfloat16)

    s_next = qk(0)
    for i in range(len(heads)):
        s_cur = s_next
        if i + 1 < len(heads):
            s_next = qk(i + 1)
        softmax_pv(i, s_cur)

    @pl.when(hs == nhs - 1)
    def _():
        for x_ref, _, _, _, wo_ref, _, o_scr, bi in branches:
            @pl.when(b == 0)
            def _():
                w_copies[2 + bi].wait()
            o_all = jnp.concatenate([o_scr[h] for h in range(n_heads)], axis=-1)
            y = jnp.dot(o_all, wo_ref[...], preferred_element_type=jnp.float32)
            out_ref[0, :, bi * d_model:(bi + 1) * d_model] = y.astype(out_ref.dtype)


@jax.jit
def pallas_concat_heads__gqa_block_cached__gqa_block_cached__near_ridge_kernel(
    A_x: jax.Array,
    A_k_cache: jax.Array,
    A_v_cache: jax.Array,
    A_wq: jax.Array,
    A_wo: jax.Array,
    B_x: jax.Array,
    B_k_cache: jax.Array,
    B_v_cache: jax.Array,
    B_wq: jax.Array,
    B_wo: jax.Array,
):
    B, Sq, D = A_x.shape
    _, Hkv, Sk, Dh = A_k_cache.shape
    Hq = A_wq.shape[1] // Dh
    assert Hq == Hkv == 32 and Dh == 192
    HPS = 2
    scale = (Dh ** -0.5) * math.log2(math.e)

    akt, avt, bkt, bvt = (jnp.swapaxes(t, 2, 3) for t in (A_k_cache, A_v_cache, B_k_cache, B_v_cache))

    x_spec = pl.BlockSpec((1, Sq, D), lambda b, h: (b, 0, 0))
    kv_spec = pl.BlockSpec((1, HPS, Dh, Sk), lambda b, h: (b, h, 0, 0))
    w_spec = pl.BlockSpec(memory_space=pl.ANY)
    out_spec = pl.BlockSpec((1, Sq, 2 * D), lambda b, h: (b, 0, 0))

    kernel = functools.partial(_attn_kernel, heads_per_step=HPS, dh=Dh, d_model=D, scale=scale)
    return pl.pallas_call(
        kernel,
        grid=(B, Hq // HPS),
        in_specs=[x_spec, kv_spec, kv_spec, w_spec, w_spec,
                  x_spec, kv_spec, kv_spec, w_spec, w_spec],
        out_specs=out_spec,
        out_shape=jax.ShapeDtypeStruct((B, Sq, 2 * D), jnp.bfloat16),
        scratch_shapes=[
            pltpu.VMEM((Hq, Sq, Dh), jnp.bfloat16),
            pltpu.VMEM((Hq, Sq, Dh), jnp.bfloat16),
            pltpu.VMEM((Hq, Sq, Dh), jnp.bfloat16),
            pltpu.VMEM((Hq, Sq, Dh), jnp.bfloat16),
            pltpu.VMEM((D, Hq * Dh), jnp.bfloat16),
            pltpu.VMEM((Hq * Dh, D), jnp.bfloat16),
            pltpu.VMEM((D, Hq * Dh), jnp.bfloat16),
            pltpu.VMEM((Hq * Dh, D), jnp.bfloat16),
            pltpu.SemaphoreType.DMA((4,)),
        ],
        compiler_params=pltpu.CompilerParams(
            dimension_semantics=("arbitrary", "arbitrary"),
            vmem_limit_bytes=100 * 1024 * 1024,
        ),
    )(A_x, akt, avt, A_wq, A_wo, B_x, bkt, bvt, B_wq, B_wo)
```
